```python
import jax
import jax.numpy as jnp

def _softmax(x, axis=-1):
    return jax.nn.softmax(x, axis=axis)

def _gelu(x):
    return jax.nn.gelu(x, approximate=True)

def _silu(x):
    return jax.nn.silu(x)

def _sigmoid(x):
    return jax.nn.sigmoid(x)

def _layernorm(x, axis=-1, eps=1e-05):
    m = jnp.mean(x, axis=axis, keepdims=True)
    v = jnp.var(x, axis=axis, keepdims=True)
    return (x - m) / jnp.sqrt(v + eps)

def _scatter_add(tgt, idx, src, axis=0):
    return tgt.at[idx].add(src)

def _segment_sum(src, seg, n):
    return jax.ops.segment_sum(src, seg, n)

class _Rng:

    def __init__(self, key):
        self._k = key

    def _next(self):
        self._k, sub = jax.random.split(self._k)
        return sub

    def normal(self, shape):
        return jax.random.normal(self._next(), shape, dtype=jnp.bfloat16)

    def randint(self, lo, hi, shape):
        return jax.random.randint(self._next(), shape, lo, hi, dtype=jnp.int32)

    def uniform(self, shape, lo=0.0, hi=1.0):
        return jax.random.uniform(self._next(), shape, jnp.bfloat16, lo, hi)

    def permutation(self, n):
        return jax.random.permutation(self._next(), n)
kernel_name = 'adaLN_cond__sliding_block_cached__dense_activation_gelu__decode'

def setup_inputs():
    _rng = _Rng(jax.random.key(int.from_bytes(__import__("os").urandom(4), "little")))
    _w = lambda a: (lambda t: t.astype(jnp.bfloat16) if jnp.issubdtype(t.dtype, jnp.floating) else t)(jnp.asarray(a))

    def _A_setup():
        B, Sq, D = (4, 1, 640)
        Hq, Hkv, Sk, Dh = (32, 32, 8192, 128)
        assert Hq % Hkv == 0, (Hq, Hkv)
        return {'x': _w((lambda *s: _rng.normal(s) * 0.05)(B, Sq, D)), 'k_cache': _w((lambda *s: _rng.normal(s) * 0.05)(B, Hkv, Sk, Dh)), 'v_cache': _w((lambda *s: _rng.normal(s) * 0.05)(B, Hkv, Sk, Dh)), 'wq': _w((lambda *s: _rng.normal(s) * 0.05)(D, Hq * Dh) * D ** (-0.5)), 'wo': _w((lambda *s: _rng.normal(s) * 0.05)(Hq * Dh, D) * (Hq * Dh) ** (-0.5))}
    _A_in = _A_setup()

    def _B_setup():
        B, S, D, F = (4, 1, 640, 1728)
        return {'x': _w((lambda *s: _rng.normal(s) * 0.05)(B, S, D)), 'w1': _w((lambda *s: _rng.normal(s) * 0.05)(D, F) * D ** (-0.5)), 'b1': _w((lambda *s: _rng.normal(s) * 0.05)(F) * 0.01), 'w2': _w((lambda *s: _rng.normal(s) * 0.05)(F, D) * F ** (-0.5)), 'b2': _w((lambda *s: _rng.normal(s) * 0.05)(D) * 0.01)}
    _B_in = _B_setup()
    return {'A_x': _A_in['x'], 'A_k_cache': _A_in['k_cache'], 'A_v_cache': _A_in['v_cache'], 'A_wq': _A_in['wq'], 'A_wo': _A_in['wo'], 'B_x': _B_in['x'], 'B_w1': _B_in['w1'], 'B_b1': _B_in['b1'], 'B_w2': _B_in['w2'], 'B_b2': _B_in['b2'], 'c': _w((lambda *s: _rng.normal(s) * 0.05)(4, 640)), 'w_mod': _w((lambda *s: _rng.normal(s) * 0.05)(640, 6 * 640) * 640 ** (-0.5))}

def reference(A_x, A_k_cache, A_v_cache, A_wq, A_wo, B_x, B_w1, B_b1, B_w2, B_b2, c, w_mod):

    def _A_ref(x, k_cache, v_cache, wq, wo):
        B, Sq, D = x.shape
        Hq, Dh = (32, 128)
        Hkv, Sk = (k_cache.shape[1], k_cache.shape[2])
        W = min(4096, max(256, Sk // 4))
        rep = Hq // Hkv
        q = (lambda x, *d: x.transpose(*d))((x @ wq).reshape(B, Sq, Hq, Dh), 0, 2, 1, 3)
        k = jnp.repeat(k_cache[:, :, Sk - W:, :], rep, axis=1)
        v = jnp.repeat(v_cache[:, :, Sk - W:, :], rep, axis=1)
        scores = jnp.einsum('bhqd,bhkd->bhqk', q, k) * Dh ** (-0.5)
        p = _softmax(scores, axis=-1)
        o = jnp.einsum('bhqk,bhkd->bhqd', p, v)
        return (lambda x, *d: x.transpose(*d))(o, 0, 2, 1, 3).reshape(B, Sq, Hq * Dh) @ wo

    def _B_ref(x, w1, b1, w2, b2):
        h = jnp.einsum('bsd,df->bsf', x, w1) + b1
        h = _gelu(h)
        return jnp.einsum('bsf,fd->bsd', h, w2) + b2
    x = A_x
    mod = (_silu(c) @ w_mod).reshape(c.shape[0], 6, 1, -1)
    sa, ca, ga, sb, cb, gb = (mod[:, 0].copy(), mod[:, 1].copy(), mod[:, 2].copy(), mod[:, 3].copy(), mod[:, 4].copy(), mod[:, 5].copy())
    h = _layernorm(x, axis=-1) * (1 + ca) + sa
    x = x + ga * _A_ref(h, A_k_cache, A_v_cache, A_wq, A_wo)
    h = _layernorm(x, axis=-1) * (1 + cb) + sb
    x = x + gb * _B_ref(h, B_w1, B_b1, B_w2, B_b2)
    return x
```

```python
import functools

import jax
import jax.numpy as jnp
from jax import lax
from jax.experimental import pallas as pl
from jax.experimental.pallas import tpu as pltpu

B, D, H, DH, SK, F = 4, 640, 32, 128, 8192, 1728
W = min(4096, max(256, SK // 4))
NSLOT = 3
RB = 128
NRB = W // RB
STAG = 4
f32, bf16 = jnp.float32, jnp.bfloat16


def _ln(x):
    m = jnp.mean(x, axis=-1, keepdims=True)
    d = x - m
    v = jnp.mean(d * d, axis=-1, keepdims=True)
    return d / jnp.sqrt(v + 1e-5)


def _mm(a, b):
    return jnp.dot(a, b, preferred_element_type=f32)


def _mm_t(a, b):
    return lax.dot_general(a, b, (((1,), (1,)), ((), ())), preferred_element_type=f32)


def _kernel(x_h, k_h, v_h, wq_h, wo_h, w1_h, b1_h, w2_h, b2_h, c_h, wm_h, o_ref,
            x_v, c_v, b1_v, b2_v, wm_v, w1_v, w2_v, kb, vb, wqb, wob, rs, ws):
    def cp(src, dst, sem, prio):
        pltpu.make_async_copy(src, dst, sem).start(priority=prio)

    def wait(dst, sem):
        pltpu.make_async_copy(dst, dst, sem).wait()

    def issue_head(g, slot, step):
        for d in (2 * step, 2 * step + 1):
            for b in range(B):
                r0 = ((d + b * STAG) % NRB) * RB
                cp(k_h.at[b, g, pl.ds(SK - W + r0, RB), :], kb.at[slot, b, pl.ds(r0, RB), :], rs.at[0, slot], 0)
                cp(v_h.at[b, g, pl.ds(SK - W + r0, RB), :], vb.at[slot, b, pl.ds(r0, RB), :], rs.at[1, slot], 1)
        col = g * DH if isinstance(g, int) else pl.multiple_of(g * DH, DH)
        if step < 5:
            cp(wq_h.at[pl.ds(step * 128, 128), pl.ds(col, DH)], wqb.at[slot, pl.ds(step * 128, 128), :], rs.at[2, slot], 0)
        if step >= 4:
            r = (step - 4) * 32
            cp(wo_h.at[pl.ds(col + r, 32), :], wob.at[slot, pl.ds(r, 32), :], rs.at[3, slot], 1)

    def issue_wm(j, lo, hi):
        for i in range(lo, hi):
            cp(wm_h.at[pl.ds(i * 16, 16), pl.ds(j * D, D)], wm_v.at[j, pl.ds(i * 16, 16), :], ws.at[j], i % 2)

    def issue_ffn(lo, hi):
        for i in range(lo, hi):
            j = min(i // 16, 4)
            cp(w1_h.at[pl.ds(i * 24, 24), :], w1_v.at[pl.ds(i * 24, 24), :], ws.at[16 + j], 0)
            cp(w2_h.at[pl.ds(i * 24, 24), :], w2_v.at[pl.ds(i * 24, 24), :], ws.at[7 + j], 1)

    tail = [functools.partial(issue_wm, j, 8 * u, 8 * u + 8) for j in range(2, 6) for u in range(5)]
    tail += [functools.partial(issue_ffn, 4 * u, 4 * u + 4) for u in range(18)]
    n30 = n31 = 16

    def spread(items, n, k):
        for it in items[(len(items) * k) // n:(len(items) * (k + 1)) // n]:
            it()

    def issue(h, step):
        @pl.when(h < H - 2)
        def _():
            issue_head(h + 2, (h + 2) % NSLOT, step)

        @pl.when(h == H - 2)
        def _():
            spread(tail[:n30], 8, step)

        @pl.when(h == H - 1)
        def _():
            spread(tail[n30:n30 + n31], 8, step)

    cp(c_h, c_v, ws.at[12], 0)
    cp(x_h, x_v, ws.at[13], 1)
    issue_wm(0, 0, 40)
    issue_wm(1, 0, 40)
    cp(b1_h, b1_v, ws.at[14], 0)
    cp(b2_h, b2_v, ws.at[15], 1)
    for s in range(8):
        issue_head(0, 0, s)
    wait(c_v, ws.at[12])
    wait(x_v, ws.at[13])
    c = c_v[...].astype(f32)
    sc = (c * jax.nn.sigmoid(c)).astype(bf16)
    x = x_v[...].astype(f32)
    lnx = _ln(x)
    wait(wm_v.at[0], ws.at[0])
    sa = _mm(sc, wm_v[0])
    wait(wm_v.at[1], ws.at[1])
    ca = _mm(sc, wm_v[1])
    hb = (lnx * (1.0 + ca) + sa).astype(bf16)
    for s in range(8):
        issue_head(1, 1, s)

    row = lax.broadcasted_iota(jnp.int32, (B, W), 0)
    rowo = lax.broadcasted_iota(jnp.int32, (B, DH), 0)

    def head(h, acc):
        slot = h % NSLOT
        wait(wqb.at[slot], rs.at[2, slot])
        q = _mm(hb, wqb[slot]).astype(bf16)
        wait(kb.at[slot], rs.at[0, slot])
        s = None
        for b in range(B):
            issue(h, b)
            sb = _mm_t(q, kb[slot, b])
            s = sb if s is None else jnp.where(row == b, sb, s)
        s = s * (DH ** -0.5)
        p = jnp.exp(s - jnp.max(s, axis=-1, keepdims=True))
        l = jnp.sum(p, axis=-1, keepdims=True)
        pb = p.astype(bf16)
        wait(vb.at[slot], rs.at[1, slot])
        o = None
        for b in range(B):
            issue(h, B + b)
            ob = _mm(pb, vb[slot, b])
            o = ob if o is None else jnp.where(rowo == b, ob, o)
        o = (o / l).astype(bf16)
        wait(wob.at[slot], rs.at[3, slot])
        return acc + _mm(o, wob[slot])

    acc = lax.fori_loop(0, H, head, jnp.zeros((B, D), f32))

    rest = tail[n30 + n31:]
    mods = []
    for j in range(2, 6):
        if j < 5:
            spread(rest, 3, j - 2)
        wait(wm_v.at[j], ws.at[j])
        mods.append(_mm(sc, wm_v[j]))
    ga, sb_, cb, gb = mods
    x1 = x + ga * acc
    h2 = (_ln(x1) * (1.0 + cb) + sb_).astype(bf16)
    wait(b1_v, ws.at[14])
    wait(b2_v, ws.at[15])
    b1 = b1_v[...].astype(f32).reshape(1, F)
    y = jnp.broadcast_to(b2_v[...].astype(f32).reshape(1, D), (B, D))
    for j in range(5):
        r0, r1 = j * 384, min(F, (j + 1) * 384)
        wait(w1_v.at[pl.ds(r0, r1 - r0), :], ws.at[16 + j])
        u = _mm_t(h2, w1_v[r0:r1, :])
        u = jax.nn.gelu(u + b1[:, r0:r1], approximate=True).astype(bf16)
        wait(w2_v.at[pl.ds(r0, r1 - r0), :], ws.at[7 + j])
        y = y + _mm(u, w2_v[r0:r1, :])
    o_ref[...] = (x1 + gb * y).astype(bf16)


@jax.jit
def pallas_adaLN_cond__sliding_block_cached__dense_activation_gelu__decode_kernel(
    A_x: jax.Array,
    A_k_cache: jax.Array,
    A_v_cache: jax.Array,
    A_wq: jax.Array,
    A_wo: jax.Array,
    B_x: jax.Array,
    B_w1: jax.Array,
    B_b1: jax.Array,
    B_w2: jax.Array,
    B_b2: jax.Array,
    c: jax.Array,
    w_mod: jax.Array,
):
    del B_x
    assert A_x.shape == (B, 1, D) and A_k_cache.shape == (B, H, SK, DH) and B_w1.shape == (D, F)
    out = pl.pallas_call(
        _kernel,
        in_specs=[pl.BlockSpec(memory_space=pltpu.HBM)] * 11,
        out_specs=pl.BlockSpec(memory_space=pltpu.VMEM),
        out_shape=jax.ShapeDtypeStruct((B, D), bf16),
        scratch_shapes=[
            pltpu.VMEM((B, D), bf16), pltpu.VMEM((B, D), bf16),
            pltpu.VMEM((F,), bf16), pltpu.VMEM((D,), bf16),
            pltpu.VMEM((6, D, D), bf16), pltpu.VMEM((F, D), bf16), pltpu.VMEM((F, D), bf16),
            pltpu.VMEM((NSLOT, B, W, DH), bf16), pltpu.VMEM((NSLOT, B, W, DH), bf16),
            pltpu.VMEM((NSLOT, D, DH), bf16), pltpu.VMEM((NSLOT, DH, D), bf16),
            pltpu.SemaphoreType.DMA((4, NSLOT)), pltpu.SemaphoreType.DMA((21,)),
        ],
        compiler_params=pltpu.CompilerParams(vmem_limit_bytes=64 * 2**20, disable_bounds_checks=True),
    )(
        A_x.reshape(B, D), A_k_cache, A_v_cache, A_wq, A_wo, B_w1.T, B_b1, B_w2, B_b2, c, w_mod,
    )
    return out.reshape(B, 1, D)
```

```python
import jax
import jax.numpy as jnp
from jax import lax
from jax.experimental import pallas as pl
from jax.experimental.pallas import tpu as pltpu

B, D, H, DH, SK, F = 4, 640, 32, 128, 8192, 1728
W = min(4096, max(256, SK // 4))
G = 4
NG = B * H // G
NSLOT = 3
RB = 64
NSTEP = 2 * G
FR = 16
FCHUNKS = (0, 768, 1408, F)
NTAIL = (5, 10)
f32, bf16 = jnp.float32, jnp.bfloat16


def _ln(x):
    m = jnp.mean(x, axis=-1, keepdims=True)
    d = x - m
    v = jnp.mean(d * d, axis=-1, keepdims=True)
    return d / jnp.sqrt(v + 1e-5)


def _mm(a, b):
    return jnp.dot(a, b, preferred_element_type=f32)


def _mm_t(a, b):
    return lax.dot_general(a, b, (((1,), (1,)), ((), ())), preferred_element_type=f32)


def _aligned(x, n):
    return x if isinstance(x, int) else pl.multiple_of(x, n)


def _kernel(x_h, k_h, v_h, wq_h, wo_h, w1_h, b1_h, w2_h, b2_h, c_h, wm_h, o_ref,
            x_v, c_v, b1_v, b2_v, wm_v, wq_v, wo_v, w1_v, w2_v, k_v, v_v,
            mod_v, q_v, acc_v, kv_sem, in_sem, wo_sem, mlp_sem):
    def cp(src, dst, sem, prio):
        pltpu.make_async_copy(src, dst, sem).start(priority=prio)

    def wait(dst, sem):
        pltpu.make_async_copy(dst, dst, sem).wait()

    def issue_group(g, slot, step):
        b, h0 = g % B, (g // B) * G
        n = W // RB // NSTEP
        for r in range(n * step * RB, n * (step + 1) * RB, RB):
            for j in range(0, G, 2):
                src = (b, pl.ds(h0 + j, 2), pl.ds(SK - W + r, RB))
                dst = (slot, pl.ds(j, 2), pl.ds(r, RB))
                cp(k_h.at[src], k_v.at[dst], kv_sem.at[0, slot], 0)
                cp(v_h.at[src], v_v.at[dst], kv_sem.at[1, slot], 1)
        if step % 2:
            rows = pl.ds(_aligned(g * DH + (step // 2) * 32, 32), 32)
            cp(wo_h.at[rows], wo_v.at[rows], wo_sem.at[g // B], 0)

    tail = [(j, r) for j in range(len(FCHUNKS) - 1) for r in range(FCHUNKS[j], FCHUNKS[j + 1], FR)]
    assert NSTEP * sum(NTAIL) >= len(tail)

    def issue_tail(items):
        for j, r in items:
            cp(w1_h.at[pl.ds(r, FR)], w1_v.at[pl.ds(r, FR)], mlp_sem.at[0, j], 0)
            cp(w2_h.at[pl.ds(r, FR)], w2_v.at[pl.ds(r, FR)], mlp_sem.at[1, j], 1)

    def issue(g, step):
        pl.when(g < NG - 2)(lambda: issue_group(g + 2, (g + 2) % NSLOT, step))
        for i in range(2):
            lo = i * NSTEP * NTAIL[0] + step * NTAIL[i]
            items = tail[lo:lo + NTAIL[i]]
            if items:
                pl.when(g == NG - 2 + i)(lambda items=items: issue_tail(items))

    def issue_weights(i, half):
        for u in range(4):
            rows = pl.ds(pl.multiple_of(u * (D // 4) + i * 8, 8), 8)
            mcols = pl.ds(half * 3 * D, 3 * D)
            qcols = pl.ds(half * H * DH // 2, H * DH // 2)
            cp(wm_h.at[rows, mcols], wm_v.at[rows, mcols], in_sem.at[0], 0)
            cp(wq_h.at[rows, qcols], wq_v.at[rows, qcols], in_sem.at[1], 1)

    lax.fori_loop(0, D // 32, lambda i, _: issue_weights(i, 0), None)
    cp(c_h, c_v, in_sem.at[2], 0)
    cp(x_h, x_v, in_sem.at[3], 1)
    cp(b1_h, b1_v, in_sem.at[4], 0)
    cp(b2_h, b2_v, in_sem.at[5], 1)
    lax.fori_loop(0, D // 32, lambda i, _: issue_weights(i, 1), None)
    for step in range(NSTEP):
        issue_group(0, 0, step)

    wait(c_v, in_sem.at[2])
    wait(x_v, in_sem.at[3])
    c = c_v[...].astype(f32)
    sc = (c * jax.nn.sigmoid(c)).astype(bf16)
    lnx = _ln(x_v[...].astype(f32))
    wait(wm_v, in_sem.at[0])
    for step in range(NSTEP):
        issue_group(1, 1, step)
        if step < 6:
            mod_v[step] = _mm(sc, wm_v[:, step * D:(step + 1) * D])
    h1 = (lnx * (1.0 + mod_v[1]) + mod_v[0]).astype(bf16)
    wait(wq_v, in_sem.at[1])
    acc_v[...] = jnp.zeros((B, D), f32)

    row_w = lax.broadcasted_iota(jnp.int32, (G, W), 0)
    row_d = lax.broadcasted_iota(jnp.int32, (G, DH), 0)
    row_b = lax.broadcasted_iota(jnp.int32, (B, DH), 0)

    def group(g, outs):
        slot, b, quad = g % NSLOT, g % B, g // B
        heads = pl.ds(pl.multiple_of(quad * G * DH, G * DH), G * DH)

        @pl.when(b == 0)
        def _():
            q_v[...] = _mm(h1, wq_v[:, heads])

        qb = q_v[pl.ds(b, 1), :]
        q = jnp.broadcast_to(qb[:, :DH], (G, DH))
        for r in range(1, G):
            q = jnp.where(row_d == r, qb[:, r * DH:(r + 1) * DH], q)
        q = q.astype(bf16)

        wait(k_v.at[slot], kv_sem.at[0, slot])
        s = None
        for r in range(G):
            issue(g, r)
            sr = _mm_t(q, k_v[slot, r])
            s = sr if s is None else jnp.where(row_w == r, sr, s)
        s = s * (DH ** -0.5)
        p = jnp.exp(s - jnp.max(s, axis=-1, keepdims=True))
        l = jnp.sum(p, axis=-1, keepdims=True)
        p = p.astype(bf16)

        wait(v_v.at[slot], kv_sem.at[1, slot])
        o = None
        for r in range(G):
            issue(g, G + r)
            o_r = _mm(p, v_v[slot, r])
            o = o_r if o is None else jnp.where(row_d == r, o_r, o)
        o = o / l
        outs = tuple(jnp.where(row_b == b, o[r:r + 1, :], outs[r]) for r in range(G))

        @pl.when(b == B - 1)
        def _():
            wait(wo_v.at[heads], wo_sem.at[quad])
            acc_v[...] += _mm(jnp.concatenate(outs, axis=1).astype(bf16), wo_v[heads, :])

        return outs

    lax.fori_loop(0, NG, group, (jnp.zeros((B, DH), f32),) * G)

    x1 = x_v[...].astype(f32) + mod_v[2] * acc_v[...]
    h2 = (_ln(x1) * (1.0 + mod_v[4]) + mod_v[3]).astype(bf16)
    wait(b1_v, in_sem.at[4])
    wait(b2_v, in_sem.at[5])
    b1 = b1_v[...].astype(f32).reshape(1, F)
    y = jnp.broadcast_to(b2_v[...].astype(f32).reshape(1, D), (B, D))
    for j in range(len(FCHUNKS) - 1):
        r0, r1 = FCHUNKS[j], FCHUNKS[j + 1]
        wait(w1_v.at[pl.ds(r0, r1 - r0)], mlp_sem.at[0, j])
        u = _mm_t(h2, w1_v[r0:r1, :]) + b1[:, r0:r1]
        u = jax.nn.gelu(u, approximate=True).astype(bf16)
        wait(w2_v.at[pl.ds(r0, r1 - r0)], mlp_sem.at[1, j])
        y = y + _mm(u, w2_v[r0:r1, :])
    o_ref[...] = (x1 + mod_v[5] * y).astype(bf16)


@jax.jit
def pallas_adaLN_cond__sliding_block_cached__dense_activation_gelu__decode_kernel(
    A_x: jax.Array,
    A_k_cache: jax.Array,
    A_v_cache: jax.Array,
    A_wq: jax.Array,
    A_wo: jax.Array,
    B_x: jax.Array,
    B_w1: jax.Array,
    B_b1: jax.Array,
    B_w2: jax.Array,
    B_b2: jax.Array,
    c: jax.Array,
    w_mod: jax.Array,
):
    del B_x
    assert A_x.shape == (B, 1, D) and B_w1.shape == (D, F)
    assert A_k_cache.shape == A_v_cache.shape == (B, H, SK, DH)
    out = pl.pallas_call(
        _kernel,
        in_specs=[pl.BlockSpec(memory_space=pltpu.HBM)] * 11,
        out_specs=pl.BlockSpec(memory_space=pltpu.VMEM),
        out_shape=jax.ShapeDtypeStruct((B, D), bf16),
        scratch_shapes=[
            pltpu.VMEM((B, D), bf16),
            pltpu.VMEM((B, D), bf16),
            pltpu.VMEM((F,), bf16),
            pltpu.VMEM((D,), bf16),
            pltpu.VMEM((D, 6 * D), bf16),
            pltpu.VMEM((D, H * DH), bf16),
            pltpu.VMEM((H * DH, D), bf16),
            pltpu.VMEM((F, D), bf16),
            pltpu.VMEM((F, D), bf16),
            pltpu.VMEM((NSLOT, G, W, DH), bf16),
            pltpu.VMEM((NSLOT, G, W, DH), bf16),
            pltpu.VMEM((6, B, D), f32),
            pltpu.VMEM((B, G * DH), f32),
            pltpu.VMEM((B, D), f32),
            pltpu.SemaphoreType.DMA((2, NSLOT)),
            pltpu.SemaphoreType.DMA((6,)),
            pltpu.SemaphoreType.DMA((H // G,)),
            pltpu.SemaphoreType.DMA((2, len(FCHUNKS) - 1)),
        ],
        compiler_params=pltpu.CompilerParams(vmem_limit_bytes=64 * 2**20),
    )(
        A_x.reshape(B, D), A_k_cache, A_v_cache, A_wq, A_wo, B_w1.T, B_b1, B_w2, B_b2, c, w_mod,
    )
    return out.reshape(B, 1, D)
```

```python
import functools

import jax
import jax.numpy as jnp
from jax import lax
from jax.experimental import pallas as pl
from jax.experimental.pallas import tpu as pltpu

B, D, H, DH, SK, F = 4, 640, 32, 128, 8192, 1728
W = min(4096, max(256, SK // 4))
G = 4
NG = B * H // G
NSLOT = 3
RB = 64
NSTEP = 2 * G
FR = 16
FCHUNKS = (0, 768, 1408, F)
WO0 = (H - G) * DH
NTAIL = (6, 10)
f32, bf16 = jnp.float32, jnp.bfloat16


def _ln(x):
    m = jnp.mean(x, axis=-1, keepdims=True)
    d = x - m
    v = jnp.mean(d * d, axis=-1, keepdims=True)
    return d / jnp.sqrt(v + 1e-5)


def _mm(a, b):
    return jnp.dot(a, b, preferred_element_type=f32)


def _mm_t(a, b):
    return lax.dot_general(a, b, (((1,), (1,)), ((), ())), preferred_element_type=f32)


def _aligned(x, n):
    return x if isinstance(x, int) else pl.multiple_of(x, n)


def _kernel(x_h, k_h, v_h, wq_h, wo_h, w1_h, b1_h, w2_h, b2_h, c_h, wm_h, o_ref,
            x_v, c_v, b1_v, b2_v, wm_v, wq_v, wo_v, w1_v, w2_v, k_v, v_v,
            mod_v, q_v, acc_v, kv_sem, in_sem, wo_sem, mlp_sem):
    def cp(src, dst, sem, prio):
        pltpu.make_async_copy(src, dst, sem).start(priority=prio)

    def wait(dst, sem):
        pltpu.make_async_copy(dst, dst, sem).wait()

    def issue_group(g, slot, step):
        b, h0 = g % B, (g // B) * G
        n = W // RB // NSTEP
        for i in range(n):
            r = _aligned((n * step + i) * RB, RB)
            for j in range(0, G, 2):
                src = (b, pl.ds(h0 + j, 2), pl.ds(SK - W + r, RB))
                dst = (slot, pl.ds(j, 2), pl.ds(r, RB))
                cp(k_h.at[src], k_v.at[dst], kv_sem.at[0, slot], 0)
                cp(v_h.at[src], v_v.at[dst], kv_sem.at[1, slot], 1)

    def issue_wo_tail(r):
        for prio in range(2):
            rows = pl.ds(WO0 + prio * (G * DH // 2) + r, FR)
            cp(wo_h.at[rows], wo_v.at[rows], wo_sem.at[1], prio)

    def issue_mlp(j, r):
        cp(w1_h.at[pl.ds(r, FR)], w1_v.at[pl.ds(r, FR)], mlp_sem.at[0, j], 0)
        cp(w2_h.at[pl.ds(r, FR)], w2_v.at[pl.ds(r, FR)], mlp_sem.at[1, j], 1)

    tail = [functools.partial(issue_wo_tail, r) for r in range(0, G * DH // 2, FR)]
    for j in range(len(FCHUNKS) - 1):
        tail += [functools.partial(issue_mlp, j, r) for r in range(FCHUNKS[j], FCHUNKS[j + 1], FR)]
    assert NSTEP * sum(NTAIL) >= len(tail)

    def issue_tail(items):
        for item in items:
            item()

    def issue(g, step):
        pl.when(g < NG - 2)(lambda: issue_group(g + 2, (g + 2) % NSLOT, step))
        for i in range(2):
            lo = i * NSTEP * NTAIL[0] + step * NTAIL[i]
            items = tail[lo:lo + NTAIL[i]]
            if items:
                pl.when(g == NG - 2 + i)(functools.partial(issue_tail, items))

    def issue_wm_wq(i, _):
        for half in range(2):
            mcols = pl.ds(half * 3 * D, 3 * D)
            qcols = pl.ds(half * H * DH // 2, H * DH // 2)
            for u in range(4):
                rows = pl.ds(pl.multiple_of(u * (D // 4) + i * 8, 8), 8)
                cp(wm_h.at[rows, mcols], wm_v.at[rows, mcols], in_sem.at[0], 0)
                cp(wq_h.at[rows, qcols], wq_v.at[rows, qcols], in_sem.at[1], 1)

    def issue_wo(i, _):
        for u in range(4):
            for prio in range(2):
                rows = pl.ds(pl.multiple_of((prio * 4 + u) * (WO0 // 8) + i * FR, FR), FR)
                cp(wo_h.at[rows], wo_v.at[rows], wo_sem.at[0], prio)

    lax.fori_loop(0, D // 4 // 8, issue_wm_wq, None)
    cp(c_h, c_v, in_sem.at[2], 0)
    cp(x_h, x_v, in_sem.at[3], 1)
    cp(b1_h, b1_v, in_sem.at[4], 0)
    cp(b2_h, b2_v, in_sem.at[5], 1)
    lax.fori_loop(0, WO0 // 8 // FR, issue_wo, None)
    lax.fori_loop(0, NSTEP, lambda step, _: issue_group(0, 0, step), None)

    wait(c_v, in_sem.at[2])
    wait(x_v, in_sem.at[3])
    c = c_v[...].astype(f32)
    sc = (c * jax.nn.sigmoid(c)).astype(bf16)
    lnx = _ln(x_v[...].astype(f32))
    wait(wm_v, in_sem.at[0])

    def modulation(step, _):
        issue_group(1, 1, step)

        @pl.when(step < 6)
        def _():
            mod_v[step] = _mm(sc, wm_v[:, pl.ds(pl.multiple_of(step * D, 128), D)])

    lax.fori_loop(0, NSTEP, modulation, None)
    h1 = (lnx * (1.0 + mod_v[1]) + mod_v[0]).astype(bf16)
    wait(wq_v, in_sem.at[1])
    wait(wo_v.at[pl.ds(0, WO0)], wo_sem.at[0])
    acc_v[...] = jnp.zeros((B, D), f32)

    row_w = lax.broadcasted_iota(jnp.int32, (G, W), 0)
    row_d = lax.broadcasted_iota(jnp.int32, (G, DH), 0)
    row_b = lax.broadcasted_iota(jnp.int32, (B, DH), 0)

    def group(g, outs):
        slot, b, quad = g % NSLOT, g % B, g // B
        heads = pl.ds(pl.multiple_of(quad * G * DH, G * DH), G * DH)

        @pl.when(b == 0)
        def _():
            q_v[...] = _mm(h1, wq_v[:, heads])

        qb = q_v[pl.ds(b, 1), :]
        q = jnp.broadcast_to(qb[:, :DH], (G, DH))
        for r in range(1, G):
            q = jnp.where(row_d == r, qb[:, r * DH:(r + 1) * DH], q)
        q = q.astype(bf16)

        wait(k_v.at[slot], kv_sem.at[0, slot])
        s = None
        for r in range(G):
            issue(g, r)
            sr = _mm_t(q, k_v[slot, r])
            s = sr if s is None else jnp.where(row_w == r, sr, s)
        s = s * (DH ** -0.5)
        p = jnp.exp(s - jnp.max(s, axis=-1, keepdims=True))
        l = jnp.sum(p, axis=-1, keepdims=True)
        p = p.astype(bf16)

        wait(v_v.at[slot], kv_sem.at[1, slot])
        o = None
        for r in range(G):
            issue(g, G + r)
            o_r = _mm(p, v_v[slot, r])
            o = o_r if o is None else jnp.where(row_d == r, o_r, o)
        o = o / l
        outs = tuple(jnp.where(row_b == b, o[r:r + 1, :], outs[r]) for r in range(G))

        @pl.when(b == B - 1)
        def _():
            pl.when(g == NG - 1)(lambda: wait(wo_v.at[pl.ds(WO0, G * DH)], wo_sem.at[1]))
            acc_v[...] += _mm(jnp.concatenate(outs, axis=1).astype(bf16), wo_v[heads, :])

        return outs

    lax.fori_loop(0, NG, group, (jnp.zeros((B, DH), f32),) * G)

    x1 = x_v[...].astype(f32) + mod_v[2] * acc_v[...]
    h2 = (_ln(x1) * (1.0 + mod_v[4]) + mod_v[3]).astype(bf16)
    wait(b1_v, in_sem.at[4])
    wait(b2_v, in_sem.at[5])
    b1 = b1_v[...].astype(f32).reshape(1, F)
    y = jnp.broadcast_to(b2_v[...].astype(f32).reshape(1, D), (B, D))
    for j in range(len(FCHUNKS) - 1):
        r0, r1 = FCHUNKS[j], FCHUNKS[j + 1]
        wait(w1_v.at[pl.ds(r0, r1 - r0)], mlp_sem.at[0, j])
        u = _mm_t(h2, w1_v[r0:r1, :]) + b1[:, r0:r1]
        u = jax.nn.gelu(u, approximate=True).astype(bf16)
        wait(w2_v.at[pl.ds(r0, r1 - r0)], mlp_sem.at[1, j])
        y = y + _mm(u, w2_v[r0:r1, :])
    o_ref[...] = (x1 + mod_v[5] * y).astype(bf16)


@jax.jit
def pallas_adaLN_cond__sliding_block_cached__dense_activation_gelu__decode_kernel(
    A_x: jax.Array,
    A_k_cache: jax.Array,
    A_v_cache: jax.Array,
    A_wq: jax.Array,
    A_wo: jax.Array,
    B_x: jax.Array,
    B_w1: jax.Array,
    B_b1: jax.Array,
    B_w2: jax.Array,
    B_b2: jax.Array,
    c: jax.Array,
    w_mod: jax.Array,
):
    del B_x
    assert A_x.shape == (B, 1, D) and B_w1.shape == (D, F)
    assert A_k_cache.shape == A_v_cache.shape == (B, H, SK, DH)
    out = pl.pallas_call(
        _kernel,
        in_specs=[pl.BlockSpec(memory_space=pltpu.HBM)] * 11,
        out_specs=pl.BlockSpec(memory_space=pltpu.VMEM),
        out_shape=jax.ShapeDtypeStruct((B, D), bf16),
        scratch_shapes=[
            pltpu.VMEM((B, D), bf16),
            pltpu.VMEM((B, D), bf16),
            pltpu.VMEM((F,), bf16),
            pltpu.VMEM((D,), bf16),
            pltpu.VMEM((D, 6 * D), bf16),
            pltpu.VMEM((D, H * DH), bf16),
            pltpu.VMEM((H * DH, D), bf16),
            pltpu.VMEM((F, D), bf16),
            pltpu.VMEM((F, D), bf16),
            pltpu.VMEM((NSLOT, G, W, DH), bf16),
            pltpu.VMEM((NSLOT, G, W, DH), bf16),
            pltpu.VMEM((6, B, D), f32),
            pltpu.VMEM((B, G * DH), f32),
            pltpu.VMEM((B, D), f32),
            pltpu.SemaphoreType.DMA((2, NSLOT)),
            pltpu.SemaphoreType.DMA((6,)),
            pltpu.SemaphoreType.DMA((2,)),
            pltpu.SemaphoreType.DMA((2, len(FCHUNKS) - 1)),
        ],
        compiler_params=pltpu.CompilerParams(vmem_limit_bytes=64 * 2**20),
    )(
        A_x.reshape(B, D), A_k_cache, A_v_cache, A_wq, A_wo, B_w1.T, B_b1, B_w2, B_b2, c, w_mod,
    )
    return out.reshape(B, 1, D)
```

```python
import functools

import jax
import jax.numpy as jnp
from jax import lax
from jax.experimental import pallas as pl
from jax.experimental.pallas import tpu as pltpu

B, D, H, DH, SK, F = 4, 640, 32, 128, 8192, 1728
W = min(4096, max(256, SK // 4))
G = 8
KC = 2
KW = W // KC
NG = B * (H // G) * KC
NSLOT = 3
RB = 64
NSTEP = 8
FR = 16
FCHUNKS = (0, 768, 1408, F)
WO0 = (H - G) * DH
NTAIL = (7, 11)
f32, bf16 = jnp.float32, jnp.bfloat16


def _ln(x):
    m = jnp.mean(x, axis=-1, keepdims=True)
    d = x - m
    v = jnp.mean(d * d, axis=-1, keepdims=True)
    return d / jnp.sqrt(v + 1e-5)


def _mm(a, b):
    return jnp.dot(a, b, preferred_element_type=f32)


def _mm_t(a, b):
    return lax.dot_general(a, b, (((1,), (1,)), ((), ())), preferred_element_type=f32)


def _aligned(x, n):
    return x if isinstance(x, int) else pl.multiple_of(x, n)


def _kernel(x_h, k_h, v_h, wq_h, wo_h, w1_h, b1_h, w2_h, b2_h, c_h, wm_h, o_ref,
            x_v, c_v, b1_v, b2_v, wm_v, wq_v, wo_v, w1_v, w2_v, k_v, v_v,
            mod_v, q_v, acc_v, kv_sem, in_sem, wo_sem, mlp_sem):
    def cp(src, dst, sem, prio):
        pltpu.make_async_copy(src, dst, sem).start(priority=prio)

    def wait(dst, sem):
        pltpu.make_async_copy(dst, dst, sem).wait()

    def issue_group(g, slot, step):
        k0, b, h0 = SK - W + (g % KC) * KW, (g // KC) % B, (g // (KC * B)) * G
        n = KW // RB // NSTEP
        for i in range(n):
            r = _aligned((n * step + i) * RB, RB)
            for j in range(0, G, 2):
                src = (b, pl.ds(h0 + j, 2), pl.ds(_aligned(k0 + r, RB), RB))
                dst = (slot, pl.ds(j, 2), pl.ds(r, RB))
                cp(k_h.at[src], k_v.at[dst], kv_sem.at[0, slot], 0)
                cp(v_h.at[src], v_v.at[dst], kv_sem.at[1, slot], 1)

    def issue_wo_tail(r):
        for prio in range(2):
            rows = pl.ds(WO0 + prio * (G * DH // 2) + r, FR)
            cp(wo_h.at[rows], wo_v.at[rows], wo_sem.at[1], prio)

    def issue_mlp(j, r):
        cp(w1_h.at[pl.ds(r, FR)], w1_v.at[pl.ds(r, FR)], mlp_sem.at[0, j], 0)
        cp(w2_h.at[pl.ds(r, FR)], w2_v.at[pl.ds(r, FR)], mlp_sem.at[1, j], 1)

    tail = [functools.partial(issue_wo_tail, r) for r in range(0, G * DH // 2, FR)]
    for j in range(len(FCHUNKS) - 1):
        tail += [functools.partial(issue_mlp, j, r) for r in range(FCHUNKS[j], FCHUNKS[j + 1], FR)]
    assert NSTEP * sum(NTAIL) >= len(tail)

    def issue_tail(items):
        for item in items:
            item()

    def issue(g, step):
        pl.when(g < NG - 2)(lambda: issue_group(g + 2, (g + 2) % NSLOT, step))
        for i in range(2):
            lo = i * NSTEP * NTAIL[0] + step * NTAIL[i]
            items = tail[lo:lo + NTAIL[i]]
            if items:
                pl.when(g == NG - 2 + i)(functools.partial(issue_tail, items))

    def issue_wm_wq(i, _):
        for half in range(2):
            mcols = pl.ds(half * 3 * D, 3 * D)
            qcols = pl.ds(half * H * DH // 2, H * DH // 2)
            for u in range(4):
                rows = pl.ds(pl.multiple_of(u * (D // 4) + i * 8, 8), 8)
                cp(wm_h.at[rows, mcols], wm_v.at[rows, mcols], in_sem.at[0], 0)
                cp(wq_h.at[rows, qcols], wq_v.at[rows, qcols], in_sem.at[1], 1)

    def issue_wo(i, _):
        for u in range(4):
            for prio in range(2):
                rows = pl.ds(pl.multiple_of((prio * 4 + u) * (WO0 // 8) + i * FR, FR), FR)
                cp(wo_h.at[rows], wo_v.at[rows], wo_sem.at[0], prio)

    lax.fori_loop(0, D // 4 // 8, issue_wm_wq, None)
    cp(c_h, c_v, in_sem.at[2], 0)
    cp(x_h, x_v, in_sem.at[3], 1)
    cp(b1_h, b1_v, in_sem.at[4], 0)
    cp(b2_h, b2_v, in_sem.at[5], 1)
    lax.fori_loop(0, WO0 // 8 // FR, issue_wo, None)
    lax.fori_loop(0, NSTEP, lambda step, _: issue_group(0, 0, step), None)

    wait(c_v, in_sem.at[2])
    wait(x_v, in_sem.at[3])
    c = c_v[...].astype(f32)
    sc = (c * jax.nn.sigmoid(c)).astype(bf16)
    lnx = _ln(x_v[...].astype(f32))
    wait(wm_v, in_sem.at[0])

    def modulation(step, _):
        issue_group(1, 1, step)

        @pl.when(step < 6)
        def _():
            mod_v[step] = _mm(sc, wm_v[:, pl.ds(pl.multiple_of(step * D, 128), D)])

    lax.fori_loop(0, NSTEP, modulation, None)
    h1 = (lnx * (1.0 + mod_v[1]) + mod_v[0]).astype(bf16)
    wait(wq_v, in_sem.at[1])
    wait(wo_v.at[pl.ds(0, WO0)], wo_sem.at[0])
    acc_v[...] = jnp.zeros((B, D), f32)

    row_w = lax.broadcasted_iota(jnp.int32, (G, KW), 0)
    row_d = lax.broadcasted_iota(jnp.int32, (G, DH), 0)
    row_b = lax.broadcasted_iota(jnp.int32, (B, DH), 0)
    hps = 2 * G // NSTEP

    def group(g, carry):
        m0, l0, o0, outs = carry
        slot, first, b, i = g % NSLOT, g % KC == 0, (g // KC) % B, g % (KC * B)
        heads = pl.ds(pl.multiple_of((g // (KC * B)) * G * DH, G * DH), G * DH)

        @pl.when(i == 0)
        def _():
            q_v[...] = _mm(h1, wq_v[:, heads])

        qb = q_v[pl.ds(b, 1), :]
        q = jnp.broadcast_to(qb[:, :DH], (G, DH))
        for r in range(1, G):
            q = jnp.where(row_d == r, qb[:, r * DH:(r + 1) * DH], q)
        q = q.astype(bf16)

        wait(k_v.at[slot], kv_sem.at[0, slot])
        s = None
        for r in range(G):
            if r % hps == 0:
                issue(g, r // hps)
            sr = _mm_t(q, k_v[slot, r])
            s = sr if s is None else jnp.where(row_w == r, sr, s)
        s = s * (DH ** -0.5)
        m0 = jnp.where(first, -jnp.inf, m0)
        m = jnp.maximum(m0, jnp.max(s, axis=-1, keepdims=True))
        shift = jnp.where(m == -jnp.inf, 0.0, m)
        p = jnp.exp(s - shift)
        alpha = jnp.exp(m0 - shift)
        l = alpha * jnp.where(first, 0.0, l0) + jnp.sum(p, axis=-1, keepdims=True)
        p = p.astype(bf16)

        wait(v_v.at[slot], kv_sem.at[1, slot])
        o = None
        for r in range(G):
            if r % hps == 0:
                issue(g, (G + r) // hps)
            o_r = _mm(p, v_v[slot, r])
            o = o_r if o is None else jnp.where(row_d == r, o_r, o)
        o = alpha * jnp.where(first, 0.0, o0) + o
        on = o / l
        outs = tuple(jnp.where(row_b == b, on[r:r + 1, :], outs[r]) for r in range(G))

        @pl.when(i == KC * B - 1)
        def _():
            pl.when(g == NG - 1)(lambda: wait(wo_v.at[pl.ds(WO0, G * DH)], wo_sem.at[1]))
            acc_v[...] += _mm(jnp.concatenate(outs, axis=1).astype(bf16), wo_v[heads, :])

        return m, l, o, outs

    stat = jnp.zeros((G, 1), f32)
    lax.fori_loop(0, NG, group, (stat, stat, jnp.zeros((G, DH), f32), (jnp.zeros((B, DH), f32),) * G))

    x1 = x_v[...].astype(f32) + mod_v[2] * acc_v[...]
    h2 = (_ln(x1) * (1.0 + mod_v[4]) + mod_v[3]).astype(bf16)
    wait(b1_v, in_sem.at[4])
    wait(b2_v, in_sem.at[5])
    b1 = b1_v[...].astype(f32).reshape(1, F)
    y = jnp.broadcast_to(b2_v[...].astype(f32).reshape(1, D), (B, D))
    for j in range(len(FCHUNKS) - 1):
        r0, r1 = FCHUNKS[j], FCHUNKS[j + 1]
        wait(w1_v.at[pl.ds(r0, r1 - r0)], mlp_sem.at[0, j])
        u = _mm_t(h2, w1_v[r0:r1, :]) + b1[:, r0:r1]
        u = jax.nn.gelu(u, approximate=True).astype(bf16)
        wait(w2_v.at[pl.ds(r0, r1 - r0)], mlp_sem.at[1, j])
        y = y + _mm(u, w2_v[r0:r1, :])
    o_ref[...] = (x1 + mod_v[5] * y).astype(bf16)


@jax.jit
def pallas_adaLN_cond__sliding_block_cached__dense_activation_gelu__decode_kernel(
    A_x: jax.Array,
    A_k_cache: jax.Array,
    A_v_cache: jax.Array,
    A_wq: jax.Array,
    A_wo: jax.Array,
    B_x: jax.Array,
    B_w1: jax.Array,
    B_b1: jax.Array,
    B_w2: jax.Array,
    B_b2: jax.Array,
    c: jax.Array,
    w_mod: jax.Array,
):
    del B_x
    assert A_x.shape == (B, 1, D) and B_w1.shape == (D, F)
    assert A_k_cache.shape == A_v_cache.shape == (B, H, SK, DH)
    out = pl.pallas_call(
        _kernel,
        in_specs=[pl.BlockSpec(memory_space=pltpu.HBM)] * 11,
        out_specs=pl.BlockSpec(memory_space=pltpu.VMEM),
        out_shape=jax.ShapeDtypeStruct((B, D), bf16),
        scratch_shapes=[
            pltpu.VMEM((B, D), bf16),
            pltpu.VMEM((B, D), bf16),
            pltpu.VMEM((F,), bf16),
            pltpu.VMEM((D,), bf16),
            pltpu.VMEM((D, 6 * D), bf16),
            pltpu.VMEM((D, H * DH), bf16),
            pltpu.VMEM((H * DH, D), bf16),
            pltpu.VMEM((F, D), bf16),
            pltpu.VMEM((F, D), bf16),
            pltpu.VMEM((NSLOT, G, KW, DH), bf16),
            pltpu.VMEM((NSLOT, G, KW, DH), bf16),
            pltpu.VMEM((6, B, D), f32),
            pltpu.VMEM((B, G * DH), f32),
            pltpu.VMEM((B, D), f32),
            pltpu.SemaphoreType.DMA((2, NSLOT)),
            pltpu.SemaphoreType.DMA((6,)),
            pltpu.SemaphoreType.DMA((2,)),
            pltpu.SemaphoreType.DMA((2, len(FCHUNKS) - 1)),
        ],
        compiler_params=pltpu.CompilerParams(vmem_limit_bytes=64 * 2**20),
    )(
        A_x.reshape(B, D), A_k_cache, A_v_cache, A_wq, A_wo, B_w1.T, B_b1, B_w2, B_b2, c, w_mod,
    )
    return out.reshape(B, 1, D)
```
